```python
import os as _os
_os.environ.setdefault("JAX_PLATFORMS", "cpu")
import jax
import jax.numpy as jnp

def _softmax(x, axis=-1):
    return jax.nn.softmax(x, axis=axis)
def _gelu(x):
    return jax.nn.gelu(x, approximate=True)
def _silu(x):
    return jax.nn.silu(x)
def _sigmoid(x):
    return jax.nn.sigmoid(x)
def _layernorm(x, axis=-1, eps=1e-5):
    m = jnp.mean(x, axis=axis, keepdims=True)
    v = jnp.var(x, axis=axis, keepdims=True)
    return (x - m) / jnp.sqrt(v + eps)
def _scatter_add(tgt, idx, src, axis=0):
    return tgt.at[idx].add(src)
def _segment_sum(src, seg, n):
    return jax.ops.segment_sum(src, seg, n)
class _Rng:
    def __init__(self, key):
        self._k = key
    def _next(self):
        self._k, sub = jax.random.split(self._k)
        return sub
    def normal(self, shape):
        return jax.random.normal(self._next(), shape, dtype=jnp.bfloat16)
    def randint(self, lo, hi, shape):
        return jax.random.randint(self._next(), shape, lo, hi, dtype=jnp.int32)
    def uniform(self, shape, lo=0.0, hi=1.0):
        return jax.random.uniform(self._next(), shape, jnp.bfloat16, lo, hi)
    def permutation(self, n):
        return jax.random.permutation(self._next(), n)


kernel_name = 'gated_mix__linear_attn_block__swiglu_ffn__prompt'

def setup_inputs():
    _rng = _Rng(jax.random.key(int.from_bytes(__import__("os").urandom(4), "little")))
    _w = (lambda a: (lambda t: t.astype(jnp.bfloat16) if jnp.issubdtype(t.dtype, jnp.floating) else t)(jnp.asarray(a)))
    def _A_setup():
        B, S, D = 1, 2048, 512
        return {
            "x": _w((lambda *s: _rng.normal(s) * 0.05)(B, S, D)),
            "wqkv": _w((lambda *s: _rng.normal(s) * 0.8)(D, 3 * D)),
            "wo": _w((lambda *s: _rng.normal(s) * 0.05)(D, D)),
        }
    _A_in = _A_setup()

    def _B_setup():
        B, S, D, F = 1, 2048, 512, 1792
        return {
            "x": _w((lambda *s: _rng.normal(s) * 0.05)(B, S, D)),
            "w_gate": _w((lambda *s: _rng.normal(s) * 0.1)(D, F)),
            "w_up": _w((lambda *s: _rng.normal(s) * 0.1)(D, F)),
            "w_down": _w((lambda *s: _rng.normal(s) * 0.1)(F, D)),
        }
    _B_in = _B_setup()

    return {
        "A_x": _A_in["x"],
        "A_wqkv": _A_in["wqkv"],
        "A_wo": _A_in["wo"],
        "B_x": _B_in["x"],
        "B_w_gate": _B_in["w_gate"],
        "B_w_up": _B_in["w_up"],
        "B_w_down": _B_in["w_down"],
        "gate_w": _w((lambda *s: _rng.normal(s) * 0.05)(512) * 16.0),
    }

def reference(A_x, A_wqkv, A_wo, B_x, B_w_gate, B_w_up, B_w_down, gate_w):
    def _A_ref(x, wqkv, wo):
        B, S, D = x.shape
        H = 32; Dh = D // H
        qkv = (lambda x, *d: x.transpose(*d))((x @ wqkv).reshape(B, S, 3, H, Dh), 2, 0, 3, 1, 4)
        q, k, v = qkv[0], qkv[1], qkv[2]
        phi = lambda t: jnp.where(t > 0, t + 1, jnp.exp(t)) + 1e-6
        pq, pk = phi(q), phi(k)
        kv = jnp.einsum("bhsd,bhse->bhde", pk, v)
        z = jnp.einsum("bhsd->bhd", pk)
        num = jnp.einsum("bhqd,bhde->bhqe", pq, kv)
        den = jnp.einsum("bhqd,bhd->bhq", pq, z)[..., None] + 1e-6
        o = num / den
        return (lambda x, *d: x.transpose(*d))(o, 0, 2, 1, 3).reshape(B, S, D) @ wo

    def _B_ref(x, w_gate, w_up, w_down):
        g = _silu(x @ w_gate)
        u = x @ w_up
        return (g * u) @ w_down

    x = A_x
    g = _sigmoid((x * gate_w).sum(-1, keepdims=True))
    a = _A_ref(x, A_wqkv, A_wo)
    b = _B_ref(x, B_w_gate, B_w_up, B_w_down)
    return g * a + (1 - g) * b
```

```python
import functools

import jax
import jax.numpy as jnp
import numpy as np
from jax import lax
import jax.experimental.pallas as pl
import jax.experimental.pallas.tpu as pltpu

S, D, F, H = 2048, 512, 1792, 32
DH = D // H
L = 128
Q = S // 4
NC = F // (2 * L)
PITCH = DH + 1
f32, bf16, i32, u32 = jnp.float32, jnp.bfloat16, jnp.int32, jnp.uint32

LHS = ((0, 3, 1), (2, 3, 1), (0, 0, 0), (3, 3, 0), (0, 1, 1), (2, 0, -1), (1, 3, -1))
RHS = ((0, 3, 1), (0, 0, 0), (1, 3, -1), (2, 0, -1), (3, 3, 0), (0, 1, 1), (2, 3, 1))
OUT = (((0, 1), (3, 1), (4, -1), (6, 1)), ((2, 1), (4, 1)),
       ((1, 1), (3, 1)), ((0, 1), (1, -1), (2, 1), (5, 1)))
RHS_IN_LHS = tuple(LHS.index(t) for t in RHS)
FLIP = (0, 1, 0, 0, 1, 1, 1)

ORD_K = (2, 4, 1, 3, 0, 5, 6)
ORD_FFN = (2, 4, 3, 0, 5, 6, 1)
ORD_IN = (2, 4, 1, 3, 0, 6, 5)
ORD_OUT = (2, 3, 4, 1, 0, 5, 6)
ORD_JIT = (2, 3, 4, 6, 0, 1, 5)


def _dot(a, b):
    return jnp.dot(a, b, preferred_element_type=f32)


def _phi(t):
    return jnp.where(t > 0, t + 1.0, jnp.exp(t)) + 1e-6


def _operand(term, quad):
    u0, u1, sign = term
    if sign == 0:
        return quad(u0)
    return quad(u0) + quad(u1) if sign > 0 else quad(u0) - quad(u1)


def _outer_operand(combine, blk):
    return [combine(lambda u: blk(2 * (u // 2) + v // 2, 2 * (u % 2) + v % 2)) for v in range(4)]


def _inner_operand(term, quads):
    return _operand(term, lambda v: quads[v]).astype(bf16)


def _result(order, prod, u):
    acc, acc_sign = None, 1
    for j, sign in sorted(OUT[u], key=lambda t: order.index(t[0])):
        if acc is None:
            acc, acc_sign = prod(j), sign
        elif acc_sign < 0:
            acc, acc_sign = prod(j) - acc, 1
        else:
            acc = acc + prod(j) if sign > 0 else acc - prod(j)
    return acc


def _ready(order, u):
    return max(order.index(j) for j, _ in OUT[u])


def _tile(j, n=1):
    return slice(j * L, (j + n) * L)


def _rows(r0, n):
    return pl.ds(r0 if isinstance(r0, int) else pl.multiple_of(r0, n), n)


def _pick(p, table):
    if isinstance(p, int):
        return table[p]
    v = table[0]
    for j in range(1, len(table)):
        v = jnp.where(p == j, table[j], v)
    return v


def _load(ref, idx, r0=0, n=L):
    return pltpu.bitcast(ref.bitcast(u32)[idx + (_rows(r0 // 2, n // 2), slice(None))], bf16)


def _take(steps, n):
    head = steps[:n]
    del steps[:n]
    return head


def _kernel(x_hbm, wqkv_hbm, wo_hbm, wg_hbm, wu_hbm, wd_hbm, gw_hbm, o_hbm,
            x_v, wqkv_v, wo_v, wg_v, wu_v, wd_v, gw_v, o_v,
            x_op, wk_op, wq_op, wf_op, wd_op, wl_op,
            wq_v, pk_v, q_v, h_v, ng_v, t_v, perm_v, mo_v, sems):
    latest = {"phase": 0}

    def issue(products, jobs=()):
        steps = [((i + 0.5) / len(s), k, f) for k, s in enumerate((products, jobs)) for i, f in enumerate(s)]
        for _, is_job, f in sorted(steps, key=lambda t: t[:2]):
            latest["phase"] += is_job
            f()

    def product(a, b):
        latest["value"] = _dot(a, b)
        return latest["value"]

    def const(value, n):
        c = int(np.float32(value).view(np.int32))
        r = latest["phase"] % 4 * (latest["value"].shape[0] // 4)
        bits = pltpu.bitcast(latest["value"][r:r + 8, :L], i32)
        return jnp.tile(pltpu.bitcast(jnp.maximum(jnp.minimum(bits, c), c), f32), (n // 8, 1))

    def placed(term, n):
        u0, u1, sign = term
        c = const(sign or 1, n)
        return lambda quad: quad(u0) + c * quad(u1) if sign else c * quad(u0)

    def selected(terms, p):
        if isinstance(p, int):
            return functools.partial(_operand, terms[p])
        u0, u1, sign = (_pick(p, [t[0] for t in terms]), _pick(p, [t[1] for t in terms]),
                        _pick(p, [float(t[2]) for t in terms]))
        return lambda quad: quad(u0) + sign * quad(u1)

    def x_rows(r0, n):
        return [(x_hbm.at[pl.ds(r0, n)], x_v.at[pl.ds(r0, n)])]

    def qkv(i, c0=0, n=D):
        return [(wqkv_hbm.at[:, pl.ds(i * D + c0, n)], wqkv_v.at[i, :, pl.ds(c0, n)])]

    def gate_up(*chunks):
        return [(w.at[:, pl.ds(c * 2 * L, 2 * L)], v.at[c]) for c in chunks
                for w, v in ((wg_hbm, wg_v), (wu_hbm, wu_v))]

    def down(r0, n):
        return [(wd_hbm.at[pl.ds(r0, n)], wd_v.at[pl.ds(r0, n)])]

    groups = [
        qkv(1, 256, 256) + x_rows(0, 256),
        qkv(1, 0, 256) + x_rows(256, 256) + [(gw_hbm, gw_v)],
        x_rows(512, 512),
        x_rows(1024, 1024),
        qkv(0) + gate_up(6) + down(0, 256),
        gate_up(0, 1) + down(256, 512),
        gate_up(2, 3, 4, 5) + down(768, 1024) + qkv(2) + [(wo_hbm, wo_v)],
    ]

    def start(g):
        for src, dst in groups[g]:
            pltpu.make_async_copy(src, dst, sems.at[g]).start()

    def wait(g):
        for src, dst in groups[g]:
            pltpu.make_async_copy(src, dst, sems.at[g]).wait()

    def copy_out(*idx):
        return pltpu.make_async_copy(o_v.at[idx], o_hbm.at[idx], sems.at[len(groups)])

    z_acc = [jnp.zeros((8, L), f32)] * 4
    delayed = []

    def run_delayed():
        while delayed:
            delayed.pop()()

    def k_slab(i):
        m = {}

        def step(p):
            if i == 0:
                w = _outer_operand(selected(RHS, p), lambda a, b: wqkv_v[1, _tile(a), _tile(b)].astype(f32))
                for v in range(4):
                    wk_op[p, v] = w[v].astype(bf16)
            xq = _outer_operand(selected(LHS, p), lambda a, b: x_v[_tile(4 * i + a), _tile(b)].astype(f32))
            for q in range(7):
                x_op[p, q, _tile(i), :] = _inner_operand(LHS[q], xq)
            half = [jnp.concatenate(xq[2 * s:2 * s + 2], axis=1) for s in range(2)]
            lhs = jnp.concatenate([half[s][r:r + 16] for r in range(0, L, 16) for s in range(2)], axis=0)
            rhs = jnp.concatenate([jnp.concatenate([_load(wk_op, (p, 2 * s + j)) for j in range(2)], axis=1)
                                   for s in range(2)], axis=0)
            o = product(lhs.astype(bf16), rhs)
            m[p] = [jnp.concatenate([o[2 * r + 16 * s:2 * r + 16 * s + 16] for r in range(0, L, 16)], axis=0)
                    for s in range(2)]
            run_delayed()
            delayed.append(functools.partial(finish, p))

        def finish(p):
            for a in range(4):
                for b in range(4):
                    u = 2 * (a // 2) + b // 2
                    if ORD_K[_ready(ORD_K, u)] == p:
                        pk = _phi(_result(ORD_K, lambda j: m[j][a % 2][:, _tile(b % 2)], u))
                        pk_v[2 * (b // 2) + a // 2, 2 * (b % 2) + a % 2, :, _tile(i)] = pk.T
                        z_acc[b] = z_acc[b] + jnp.sum(pk.reshape(L // 8, 8, L), axis=0)

        return [functools.partial(step, p) for p in ORD_K]

    def gate_jobs(gw):
        def job(i, a):
            w = jnp.tile(jnp.tile(const(0.5, 8), (1, 4)) * gw, (L // 8, 1))
            s = jnp.sum(x_v[_tile(4 * i + a), :].astype(f32) * w, axis=-1, keepdims=True)
            ng_v[a, _tile(i), :] = jnp.broadcast_to(0.5 - 0.5 * jnp.tanh(s), (L, L))
        return [functools.partial(job, i, a) for i in range(4) for a in range(4)]

    def put_heads(ref, k, rows, h0=0):
        for h in range(rows.shape[0] // DH):
            ref[k, pl.ds((h0 + h) * PITCH, DH), :] = rows[h * DH:(h + 1) * DH]

    def reorder_columns(k, words):
        put_heads(perm_v, k, words.T)
        return jnp.concatenate([perm_v[k, pl.ds(d, H, stride=PITCH), :] for d in range(DH)], axis=0).T

    def reorder_wq():
        words = pltpu.bitcast(wqkv_v[0], u32)
        for k in range(2):
            w = reorder_columns(k, words[_tile(k)])
            for j in range(2):
                wq_v[2 * k + j] = w[:, _tile(2 * j, 2)]

    def q_part(p, slot, r0, n, prepare):
        m = {}

        def step(q):
            if prepare and not m:
                rule = selected(RHS, p)
                w = [rule(lambda u: pltpu.bitcast(wq_v[u, pl.ds(v // 2 * 64, 64), _tile(v % 2)], bf16).astype(f32))
                     for v in range(4)]
                for j in ORD_IN:
                    wq_op[slot, j] = _inner_operand(RHS[j], w)
            m[q] = product(_load(x_op, (p, q), r0, n), _load(wq_op, (slot, q)))
            if len(m) == 7:
                for v in range(4):
                    q_v[p, v, r0:r0 + n, :] = _result(ORD_IN, m.get, v)

        return [functools.partial(step, q) for q in ORD_IN]

    def normalize_jobs(r0, z):
        def job(r, s):
            rows = _rows(r0 + r, 8)
            one = const(1, 8)
            m = [q_v[p, 2 * s:2 * s + 2, rows, :] for p in range(7)]
            m[2], m[3] = m[2] * one, m[3] * one
            for a in (s, s + 2):
                pq = [_phi(_result((2, 3, 0, 1, 4, 5, 6), lambda p: m[p][b % 2], 2 * (a // 2) + b // 2))
                      for b in range(4)]
                den = (pq[0] * z[0] + pq[1] * z[1]) + (pq[2] * z[2] + pq[3] * z[3])
                den = den + pltpu.roll(den, 2 * H, 1)
                den = den + pltpu.roll(den, H, 1)
                scale = pl.reciprocal(den + 1e-6, full_range=False) * (1.0 - ng_v[a, rows, :])
                h_v[a, 2 * NC:, rows, :] = jnp.stack([t * scale for t in pq])
        return [functools.partial(job, r, s) for r in range(0, L, 8) for s in range(2)]

    def t_part(p):
        rule, px = selected(LHS, p), _pick(p, RHS_IN_LHS)
        quads = [rule(lambda u: pk_v[u, v]) for v in range(4)]
        m = {}

        def step(q):
            m[q] = _dot(_inner_operand(LHS[q], quads), _load(x_op, (px, RHS_IN_LHS[q]), 0, Q))
            if len(m) == 7:
                for v in sorted(range(4), key=lambda v: _ready(ORD_JIT, v)):
                    t_v[p, v] = _result(ORD_JIT, m.get, v)

        return [functools.partial(step, q) for q in ORD_JIT]

    kv = {}

    def kv_step(a):
        t = jnp.concatenate([_result(ORD_FFN, lambda p: t_v[p, 2 * (a % 2) + b % 2], 2 * (a // 2) + b // 2)
                             for b in range(4)], axis=1)
        same_head = (lax.broadcasted_iota(i32, (L, L), 0) // DH) == (lax.broadcasted_iota(i32, (L, L), 1) // DH)
        kv[a] = jnp.where(same_head, product(t.astype(bf16), wqkv_v[2, :, _tile(a)]), 0.0).astype(bf16)

    def mo_step(a):
        mo = product(kv[a], wo_v[_tile(a), :])
        for b in range(4):
            put_heads(mo_v, b, mo[:, _tile(b)], a * L // DH)

    def balance():
        mag = [jnp.sum(jnp.sum(jnp.abs(w[NC - 1, :L, :].astype(f32)), axis=0, keepdims=True), axis=1, keepdims=True)
               for w in (wg_v, wu_v)]
        bg, bu = [pltpu.bitcast(jnp.broadcast_to(t, (8, L)), i32) >> 1 for t in mag]
        shift = jnp.clip((bu - bg + (1 << 21)) >> 22, -40, 40) << 23
        return pltpu.bitcast(0x3F800000 + shift, f32)[:1], pltpu.bitcast(0x3F000000 - shift, f32)[:1]

    def ffn_part(c, slot, r0, n, prepare):
        m = {}

        def weight(a, b):
            w = (wg_v, wu_v)[b // 2][c, _tile(a), _tile(b % 2)].astype(f32)
            return w if b // 2 else w * wg_scale

        def step(p, q):
            if prepare and q == ORD_IN[0]:
                w = _outer_operand(selected(RHS, p), weight)
                for j in ORD_IN:
                    wf_op[slot, p, j] = _inner_operand(RHS[j], w)
            m[p, q] = product(_load(x_op, (p, q), r0, n), _load(wf_op, (slot, p, q)))
            if len(m) == 49:
                inner = [[_result(ORD_IN, lambda j: m[i, j], v) for v in range(4)] for i in range(7)]
                for a in range(4):
                    for b in range(2):
                        gate, up = [_result(ORD_FFN, lambda i: inner[i][2 * (a % 2) + b], 2 * (a // 2) + k)
                                    for k in range(2)]
                        t = half_unscale * gate
                        h_v[a, 2 * c + b, r0:r0 + n, :] = (t + t * jnp.tanh(t)) * (up * ng_v[a, r0:r0 + n, :])

        return [functools.partial(step, p, q) for p in ORD_FFN for q in ORD_IN]

    def down_jobs(dst, n, blk):
        def job(p, r):
            w = _outer_operand(placed(RHS[p], 16), lambda a, b: blk(a, b ^ FLIP[p], r))
            wd_op[p, :, _rows(dst + r, 16), :] = jnp.stack([_inner_operand(t, w) for t in RHS])
        return [functools.partial(job, p, r) for p in ORD_OUT for r in range(0, n, 16)]

    def wd_jobs(c):
        src = 2 * L + (c >> 1) * 4 * L + (c & 1) * 64
        return down_jobs(c * 64, 64, lambda a, b, r: wd_v[_rows(src + a * L + r, 16), _tile(b)].astype(f32))

    def mo_jobs():
        return down_jobs(3 * L, L, lambda a, b, r: mo_v[b, pl.ds(4 * a + r // H + r % H * PITCH, 16, stride=PITCH), :])

    def wd_first_jobs():
        def job(p, r):
            rule = placed(RHS[p], 64)
            for j in range(2):
                w = rule(lambda u: wd_v[pl.ds(u // 2 * L + r, 64), _tile(2 * (u % 2) + j)].astype(f32))
                wl_op[p, j, r:r + 64, :] = w.astype(bf16)
        return [functools.partial(job, p, r) for p in range(7) for r in (0, 64)]

    def out_slab(i, send=False):
        rows = _rows(i * L, L)
        m, quads, inner = {}, {}, {}

        def first(p):
            lhs = [_operand(LHS[p], lambda u: h_v[2 * (u // 2) + s, u % 2, rows, :]) for s in range(2)]
            m[p] = product(jnp.concatenate(lhs, axis=0).astype(bf16),
                           jnp.concatenate([_load(wl_op, (p, j)) for j in range(2)], axis=1))
            quads[p] = _outer_operand(selected(LHS, p), lambda a, b: jnp.concatenate(
                [h_v[a, 2 + 4 * t + b, rows, :] for t in range(4)], axis=1))

        def step(p, q):
            m[p, q] = product(_inner_operand(LHS[q], quads[p]), _load(wd_op, (p, q), 0, 4 * L))
            if q != ORD_JIT[-1]:
                return
            inner[p] = [_result(ORD_JIT, lambda j: m[p, j], v ^ FLIP[p]) + m[p][_tile(v // 2), _tile(v % 2)]
                        for v in range(4)]
            for u in range(4):
                if ORD_OUT[_ready(ORD_OUT, u)] == p:
                    for s in range(2):
                        o = [_result(ORD_OUT, lambda k: inner[k][2 * s + j], u) for j in range(2)]
                        idx = (_rows((4 * i + 2 * (u // 2) + s) * L, L), pl.ds(u % 2 * 2 * L, 2 * L))
                        o_v[idx] = jnp.concatenate(o, axis=1).astype(bf16)
                        if send:
                            copy_out(*idx).start()

        return [f for p in ORD_OUT
                for f in [functools.partial(first, p)] + [functools.partial(step, p, q) for q in ORD_JIT]]

    for g in range(6):
        start(g)
    k = [f for i in range(4) for f in k_slab(i)]
    wait(0)
    issue(_take(k, 2))
    wait(1)
    gates = gate_jobs(jnp.broadcast_to(gw_v[...].astype(f32).reshape(1, D), (8, D)))

    def k_and_gates(*counts):
        for n, ng in counts:
            issue(_take(k, n) + _take(gates, ng))

    k_and_gates((1, 1), (2, 1), (2, 0))
    wait(2)
    k_and_gates((1, 2), (2, 2), (2, 2), (2, 0))
    wait(3)
    k_and_gates((1, 2), (2, 2), (2, 2), (3, 2), (2, 0))
    wait(4)
    start(6)
    wg_scale, half_unscale = balance()
    reorder_wq()
    issue(k)
    run_delayed()
    ffn = ffn_part(6, 2, 0, 256, True)
    issue(_take(ffn, 12))
    issue(_take(ffn, 24), wd_first_jobs())
    issue(ffn + t_part(6))
    wait(5)

    def chunk_pair(i, _):
        pl.when(i == 1)(lambda: wait(6))
        for slot in range(2):
            c = 2 * i + slot
            t = t_part(c)
            issue(_take(t, 2) + ffn_part(c, slot, 0, 256, True) + q_part(c, slot, 0, 256, True))
            ffn = ffn_part(c, slot, 256, 256, False)
            issue(_take(ffn, 24), wd_jobs(c))
            issue(ffn + q_part(c, slot, 256, 256, False) + t)

    lax.fori_loop(0, 3, chunk_pair, None)

    z = jnp.sum(jnp.concatenate(z_acc, axis=1), axis=0, keepdims=True)
    z = pltpu.bitcast(reorder_columns(2, pltpu.bitcast(jnp.broadcast_to(z, (L, D)), u32))[:8], f32)
    z = [z[:, _tile(b)] for b in range(4)]
    norm, mo = normalize_jobs(0, z), mo_jobs()
    ffn = ffn_part(6, 2, 256, 256, False)
    kvs = [functools.partial(kv_step, a) for a in range(4)]
    issue(kvs + q_part(6, 2, 0, L, True))
    issue([functools.partial(mo_step, a) for a in range(4)], _take(norm, 12))
    issue(q_part(6, 2, L, L, False), _take(norm, 5))
    issue(_take(ffn, 16), norm)
    issue(_take(ffn, 20), _take(mo, 40))
    rest = q_part(6, 2, 2 * L, 2 * L, False)
    issue(ffn + _take(rest, 3))
    issue(rest, mo)

    def slab(i, _):
        out, norm = out_slab(i), normalize_jobs((i + 1) * L, z)
        issue(_take(out, 1))
        issue(_take(out, 15), _take(norm, 18))
        issue(_take(out, 28), norm)
        issue(out)

    lax.fori_loop(0, 3, slab, None)

    out = out_slab(3, send=True)
    issue(_take(out, 2))
    copy_out(pl.ds(0, 12 * L)).start()
    issue(out)
    copy_out(pl.ds(0, S)).wait()


@jax.jit
def pallas_gated_mix__linear_attn_block__swiglu_ffn__prompt_kernel(
    A_x: jax.Array,
    A_wqkv: jax.Array,
    A_wo: jax.Array,
    B_x: jax.Array,
    B_w_gate: jax.Array,
    B_w_up: jax.Array,
    B_w_down: jax.Array,
    gate_w: jax.Array,
):
    del B_x
    hbm = pl.BlockSpec(memory_space=pltpu.HBM)
    vmem = pltpu.VMEM
    out = pl.pallas_call(
        _kernel,
        out_shape=jax.ShapeDtypeStruct((S, D), bf16),
        in_specs=[hbm] * 7,
        out_specs=hbm,
        scratch_shapes=[
            vmem((S, D), bf16), vmem((3, D, D), bf16), vmem((D, D), bf16),
            vmem((NC, D, 2 * L), bf16), vmem((NC, D, 2 * L), bf16), vmem((F, D), bf16),
            vmem((D,), bf16), vmem((S, D), bf16),
            vmem((7, 7, Q, L), bf16),
            vmem((7, 4, L, L), bf16),
            vmem((3, 7, L, L), bf16),
            vmem((3, 7, 7, L, L), bf16),
            vmem((7, 7, 4 * L, L), bf16),
            vmem((7, 2, L, L), bf16),
            vmem((4, L, 2 * L), u32),
            vmem((4, 4, L, Q), f32),
            vmem((7, 4, Q, L), f32),
            vmem((4, 2 * NC + 4, Q, L), f32),
            vmem((4, Q, L), f32),
            vmem((7, 4, L, L), f32),
            vmem((3, H * PITCH + DH, L), u32),
            vmem((4, H * PITCH + DH, L), f32),
            pltpu.SemaphoreType.DMA((8,)),
        ],
        compiler_params=pltpu.CompilerParams(vmem_limit_bytes=100 * 1024 * 1024),
    )(A_x.reshape(S, D), A_wqkv, A_wo, B_w_gate, B_w_up, B_w_down, gate_w)
    return out.reshape(1, S, D)
```
